```python
import jax
import jax.numpy as jnp

def _softmax(x, axis=-1):
    return jax.nn.softmax(x, axis=axis)
def _gelu(x):
    return jax.nn.gelu(x, approximate=True)
def _silu(x):
    return jax.nn.silu(x)
def _sigmoid(x):
    return jax.nn.sigmoid(x)
def _layernorm(x, axis=-1, eps=1e-5):
    m = jnp.mean(x, axis=axis, keepdims=True)
    v = jnp.var(x, axis=axis, keepdims=True)
    return (x - m) / jnp.sqrt(v + eps)
def _scatter_add(tgt, idx, src, axis=0):
    return tgt.at[idx].add(src)
def _segment_sum(src, seg, n):
    return jax.ops.segment_sum(src, seg, n)
class _Rng:
    def __init__(self, key):
        self._k = key
    def _next(self):
        self._k, sub = jax.random.split(self._k)
        return sub
    def normal(self, shape):
        return jax.random.normal(self._next(), shape, dtype=jnp.bfloat16)
    def randint(self, lo, hi, shape):
        return jax.random.randint(self._next(), shape, lo, hi, dtype=jnp.int32)
    def uniform(self, shape, lo=0.0, hi=1.0):
        return jax.random.uniform(self._next(), shape, jnp.bfloat16, lo, hi)
    def permutation(self, n):
        return jax.random.permutation(self._next(), n)


kernel_name = 'standalone__layernorm_linear__prompt'

def setup_inputs():
    _rng = _Rng(jax.random.key(int.from_bytes(__import__("os").urandom(4), "little")))
    _w = (lambda a: (lambda t: t.astype(jnp.bfloat16) if jnp.issubdtype(t.dtype, jnp.floating) else t)(jnp.asarray(a)))
    B, S, D = 2, 2048, 1024
    return {
        "x": _w((lambda *s: _rng.normal(s) * 0.05)(B, S, D)),
        "g": _w((lambda *s: _rng.normal(s) * 0.05)(D) + 1.0),
        "b": _w((lambda *s: _rng.normal(s) * 0.05)(D)),
        "w": _w((lambda *s: _rng.normal(s) * 0.05)(D, D)),
    }

def reference(x, g, b, w):
    return (_layernorm(x, axis=-1) * g + b) @ w
```

```python
import jax
import jax.numpy as jnp
import jax.experimental.pallas as pl
import jax.experimental.pallas.tpu as pltpu

_EPS = 1e-5

_X0 = (128, 128, 128)
_WK = (128, 256, 256, 384)
_XS = (192, 384, 768, 1536, 832)
_XW = (None, 384, 576, 960, 1728)
_DEFER_OUT_UNTIL = 4
_MM_ROWS = 512
_LN_ROWS = 512
_TAIL = ((128, 1), (128, 4))


def _plan(n_rows, d):
    plan = []
    r0 = sum(_X0)
    assert r0 + sum(_XS) == n_rows and sum(_WK) == d
    xr = [r0 + sum(_XS[:i]) for i in range(len(_XS))]
    wk = [sum(_WK[:i]) for i in range(len(_WK))]

    def norm(a, n):
        for q in range(0, n, _LN_ROWS):
            plan.append(("norm", a + q, min(_LN_ROWS, n - q)))

    plan.append(("start_gb",))
    o = 0
    for i, n in enumerate(_X0):
        plan.append(("start_x", ("first", i), o, n))
        o += n
    plan.append(("wait_gb",))
    for j in range(len(_WK)):
        plan.append(("start_w", j, wk[j], _WK[j]))
    o = 0
    for i, n in enumerate(_X0):
        plan.append(("wait_x", ("first", i)))
        if i == 0:
            for q in range(len(_XS)):
                plan.append(("start_x", q, xr[q], _XS[q]))
        norm(o, n)
        o += n

    outs = []
    n_out = 0
    deferring = True

    def emit_out(*a):
        nonlocal n_out
        outs.append(("start_out", n_out) + a)
        n_out += 1
        if not deferring:
            plan.extend(outs)
            outs.clear()

    def wait_rows(q):
        nonlocal deferring
        plan.append(("wait_x", q))
        if q == _DEFER_OUT_UNTIL:
            deferring = False
            plan.extend(outs)
            outs.clear()
        norm(xr[q], _XS[q])

    for j in range(len(_WK)):
        plan.append(("wait_w", j))
        if j == len(_WK) - 1:
            for q in range(len(_XS)):
                if _XW[q] is None:
                    wait_rows(q)
        plan.append(("matmul_k", r0, wk[j], _WK[j], j == 0, j == len(_WK) - 1))
    emit_out(0, r0, 0, d)

    n_tail = sum(t[0] for t in _TAIL)
    bounds = sorted({r0, n_rows - n_tail} | set(xr) | {w for w in _XW if w is not None})
    for a, b in zip(bounds[:-1], bounds[1:]):
        nt = -(-(b - a) // _MM_ROWS)
        base = (b - a) // nt // 16 * 16
        q = a
        for t in range(nt):
            s = base if t < nt - 1 else b - q
            for i in range(len(_XS)):
                if _XW[i] == q:
                    wait_rows(i)
            plan.append(("matmul", q, s, 0, d))
            emit_out(q, s, 0, d)
            q += s
    a = n_rows - n_tail
    for s, parts in _TAIL:
        nc = d // parts
        for j in range(parts):
            plan.append(("matmul", a, s, j * nc, nc))
            emit_out(a, s, j * nc, nc)
        a += s
    assert not outs
    for q in range(n_out):
        plan.append(("wait_out", q))
    return plan, n_out


@jax.jit
def pallas_standalone__layernorm_linear__prompt_kernel(
    x: jax.Array,
    g: jax.Array,
    b: jax.Array,
    w: jax.Array,
):
    bsz, seq, d = x.shape
    m = bsz * seq
    plan, n_out = _plan(m, d)
    n_x = len(_X0) + len(_XS)
    r0 = sum(_X0)

    def kernel_function(x_hbm, g_hbm, b_hbm, w_hbm, o_hbm,
                        x_vmem, w_vmem, y_vmem, o_vmem, acc_vmem, g_vmem, b_vmem,
                        x_sem, w_sem, o_sem, gb_sem):
        copies = {}
        gb = []
        x_slot = {}
        for step in plan:
            kind = step[0]
            if kind == "start_gb":
                copies["g"] = pltpu.make_async_copy(g_hbm, g_vmem, gb_sem.at[0])
                copies["b"] = pltpu.make_async_copy(b_hbm, b_vmem, gb_sem.at[1])
                copies["g"].start()
                copies["b"].start()
            elif kind == "wait_gb":
                copies["g"].wait()
                copies["b"].wait()
                gb.append(g_vmem[...].astype(jnp.float32).reshape(1, d))
                gb.append(b_vmem[...].astype(jnp.float32).reshape(1, d))
            elif kind == "start_x":
                _, key, a, n = step
                x_slot[key] = len(x_slot)
                copies["x", key] = pltpu.make_async_copy(
                    x_hbm.at[pl.ds(a, n)], x_vmem.at[pl.ds(a, n)], x_sem.at[x_slot[key]])
                copies["x", key].start(priority=1)
            elif kind == "wait_x":
                copies["x", step[1]].wait()
            elif kind == "start_w":
                _, j, k0, nk = step
                copies["w", j] = pltpu.make_async_copy(
                    w_hbm.at[pl.ds(k0, nk)], w_vmem.at[pl.ds(k0, nk)], w_sem.at[j])
                copies["w", j].start(priority=1)
            elif kind == "wait_w":
                copies["w", step[1]].wait()
            elif kind == "start_out":
                _, i, a, n, c0, nc = step
                if nc == d:
                    src, dst = o_vmem.at[pl.ds(a, n)], o_hbm.at[pl.ds(a, n)]
                else:
                    src = o_vmem.at[pl.ds(a, n), pl.ds(c0, nc)]
                    dst = o_hbm.at[pl.ds(a, n), pl.ds(c0, nc)]
                copies["o", i] = pltpu.make_async_copy(src, dst, o_sem.at[i])
                copies["o", i].start(priority=1)
            elif kind == "wait_out":
                copies["o", step[1]].wait()
            elif kind == "norm":
                _, a, n = step
                xf = x_vmem[pl.ds(a, n), :].astype(jnp.float32)
                mean = jnp.sum(xf, axis=-1, keepdims=True) * (1.0 / d)
                xc = xf - mean
                var = jnp.sum(xc * xc, axis=-1, keepdims=True) * (1.0 / d)
                y = xc * jax.lax.rsqrt(var + _EPS) * gb[0] + gb[1]
                y_vmem[pl.ds(a, n), :] = y.astype(y_vmem.dtype)
            elif kind == "matmul_k":
                _, n, k0, nk, first, last = step
                p = jnp.dot(y_vmem[pl.ds(0, n), k0:k0 + nk], w_vmem[k0:k0 + nk, :],
                            preferred_element_type=jnp.float32)
                if not first:
                    p = p + acc_vmem[...]
                if last:
                    o_vmem[pl.ds(0, n), :] = p.astype(o_vmem.dtype)
                else:
                    acc_vmem[...] = p
            elif kind == "matmul":
                _, a, n, c0, nc = step
                p = jnp.dot(y_vmem[pl.ds(a, n), :], w_vmem[:, c0:c0 + nc],
                            preferred_element_type=jnp.float32)
                o_vmem[pl.ds(a, n), c0:c0 + nc] = p.astype(o_vmem.dtype)
            else:
                raise ValueError(kind)

    out = pl.pallas_call(
        kernel_function,
        in_specs=[pl.BlockSpec(memory_space=pl.ANY)] * 4,
        out_specs=pl.BlockSpec(memory_space=pl.ANY),
        out_shape=jax.ShapeDtypeStruct((m, d), x.dtype),
        scratch_shapes=[
            pltpu.VMEM((m, d), x.dtype),
            pltpu.VMEM((d, d), w.dtype),
            pltpu.VMEM((m, d), w.dtype),
            pltpu.VMEM((m, d), x.dtype),
            pltpu.VMEM((r0, d), jnp.float32),
            pltpu.VMEM((d,), g.dtype),
            pltpu.VMEM((d,), b.dtype),
            pltpu.SemaphoreType.DMA((n_x,)),
            pltpu.SemaphoreType.DMA((len(_WK),)),
            pltpu.SemaphoreType.DMA((n_out,)),
            pltpu.SemaphoreType.DMA((2,)),
        ],
        compiler_params=pltpu.CompilerParams(
            vmem_limit_bytes=100 * 1024 * 1024,
            flags={"XLA_TPU_EVENLY_DISTRIBUTE_CRITICAL_NODES": True},
        ),
    )(x.reshape(m, d), g, b, w)
    return out.reshape(bsz, seq, d)
```

```python
import jax
import jax.numpy as jnp
import jax.experimental.pallas as pl
import jax.experimental.pallas.tpu as pltpu

_EPS = 1e-5

_X0 = (128, 128, 64)
_WK = (128, 128, 256, 256, 256)
_XS = (256, 256, 576, 704, 704, 832, 448)
_TAIL = ((64, 1), (64, 2))
_PREP_ROWS = 32
_T_ROWS = 8


def _plan(n_rows, d):
    plan = []
    r0 = sum(_X0)
    assert r0 + sum(_XS) == n_rows and sum(_WK) == d
    xr = [r0 + sum(_XS[:i]) for i in range(len(_XS))]
    wk = [sum(_WK[:i]) for i in range(len(_WK))]
    n_tail = sum(t[0] for t in _TAIL)
    assert _XS[-1] > n_tail

    plan.append(("start_gb",))
    o = 0
    for i, n in enumerate(_X0):
        plan.append(("start_x", ("first", i), o, n))
        o += n
    plan.append(("wait_gb",))
    for j in range(len(_WK)):
        plan.append(("start_w", j, wk[j], _WK[j]))
    o = 0
    for i, n in enumerate(_X0):
        plan.append(("wait_x", ("first", i)))
        if i == 0:
            for q in range(len(_XS)):
                plan.append(("start_x", q, xr[q], _XS[q]))
        plan.append(("norm", o, n))
        o += n

    tiles = [[(a, n, None)] for a, n in zip(xr, _XS)]
    tiles[-1] = [(xr[-1], _XS[-1] - n_tail, None)]
    a = n_rows - n_tail
    for n, parts in _TAIL:
        tiles[-1].append((a, n, parts))
        a += n

    outs = []
    n_out = 0
    deferring = True

    def emit_out(*a):
        nonlocal n_out
        outs.append(("start_out", n_out) + a)
        n_out += 1
        if not deferring:
            plan.extend(outs)
            outs.clear()

    def wait_rows(q):
        nonlocal deferring
        plan.append(("wait_x", q))
        if q == len(_XS) - 1:
            deferring = False
            plan.extend(outs)
            outs.clear()
        for a, n, parts in tiles[q]:
            plan.append(("norm", a, n) if parts else ("norm_sums", a, n))

    for j in range(len(_WK)):
        plan.append(("wait_w", j))
        if j == len(_WK) - 1:
            wait_rows(0)
            plan.append(("w_sums",))
        plan.append(("matmul_k", r0, wk[j], _WK[j], j == 0, j == len(_WK) - 1))
    emit_out(0, r0, 0, d)

    for i in range(len(_XS)):
        if i + 1 < len(_XS):
            wait_rows(i + 1)
        for a, n, parts in tiles[i]:
            if parts is None:
                plan.append(("strassen", a, n))
                emit_out(a, n, 0, d)
            else:
                nc = d // parts
                for j in range(parts):
                    plan.append(("matmul", a, n, j * nc, nc))
                    emit_out(a, n, j * nc, nc)
    assert not outs
    for q in range(n_out):
        plan.append(("wait_out", q))
    return plan, n_out


@jax.jit
def pallas_standalone__layernorm_linear__prompt_kernel(
    x: jax.Array,
    g: jax.Array,
    b: jax.Array,
    w: jax.Array,
):
    bsz, seq, d = x.shape
    m = bsz * seq
    h = d // 2
    plan, n_out = _plan(m, d)
    n_x = len(_X0) + len(_XS)
    r0 = sum(_X0)
    f32 = jnp.float32
    mxu = w.dtype

    def kernel_function(x_hbm, g_hbm, b_hbm, w_hbm, o_hbm,
                        x_vmem, w_vmem, y_vmem, o_vmem, acc_vmem, t_vmem, s_vmem,
                        g_vmem, b_vmem, x_sem, w_sem, o_sem, gb_sem):
        copies = {}
        gb = []
        x_slot = {}

        def norm(a, n):
            xf = x_vmem[pl.ds(a, n), :].astype(f32)
            mean = jnp.sum(xf, axis=-1, keepdims=True) * (1.0 / d)
            xc = xf - mean
            var = jnp.sum(xc * xc, axis=-1, keepdims=True) * (1.0 / d)
            return xc * jax.lax.rsqrt(var + _EPS) * gb[0] + gb[1]

        for step in plan:
            kind = step[0]
            if kind == "start_gb":
                copies["g"] = pltpu.make_async_copy(g_hbm, g_vmem, gb_sem.at[0])
                copies["b"] = pltpu.make_async_copy(b_hbm, b_vmem, gb_sem.at[1])
                copies["g"].start()
                copies["b"].start()
            elif kind == "wait_gb":
                copies["g"].wait()
                copies["b"].wait()
                gb.append(g_vmem[...].astype(f32).reshape(1, d))
                gb.append(b_vmem[...].astype(f32).reshape(1, d))
            elif kind == "start_x":
                _, key, a, n = step
                x_slot[key] = len(x_slot)
                copies["x", key] = pltpu.make_async_copy(
                    x_hbm.at[pl.ds(a, n)], x_vmem.at[pl.ds(a, n)], x_sem.at[x_slot[key]])
                copies["x", key].start(priority=1)
            elif kind == "wait_x":
                copies["x", step[1]].wait()
            elif kind == "start_w":
                _, j, k0, nk = step
                copies["w", j] = pltpu.make_async_copy(
                    w_hbm.at[pl.ds(k0, nk)], w_vmem.at[pl.ds(k0, nk)], w_sem.at[j])
                copies["w", j].start(priority=1)
            elif kind == "wait_w":
                copies["w", step[1]].wait()
            elif kind == "start_out":
                _, i, a, n, c0, nc = step
                if nc == d:
                    src, dst = o_vmem.at[pl.ds(a, n)], o_hbm.at[pl.ds(a, n)]
                else:
                    src = o_vmem.at[pl.ds(a, n), pl.ds(c0, nc)]
                    dst = o_hbm.at[pl.ds(a, n), pl.ds(c0, nc)]
                copies["o", i] = pltpu.make_async_copy(src, dst, o_sem.at[i])
                copies["o", i].start(priority=1)
            elif kind == "wait_out":
                copies["o", step[1]].wait()
            elif kind == "norm":
                _, a, n = step
                y_vmem[pl.ds(a, n), :] = norm(a, n).astype(mxu)
            elif kind == "matmul_k":
                _, n, k0, nk, first, last = step
                p = jnp.dot(y_vmem[pl.ds(0, n), k0:k0 + nk], w_vmem[k0:k0 + nk, :],
                            preferred_element_type=f32)
                if not first:
                    p = p + acc_vmem[...]
                if last:
                    o_vmem[pl.ds(0, n), :] = p.astype(o_vmem.dtype)
                else:
                    acc_vmem[...] = p
            elif kind == "matmul":
                _, a, n, c0, nc = step
                p = jnp.dot(y_vmem[pl.ds(a, n), :], w_vmem[:, c0:c0 + nc],
                            preferred_element_type=f32)
                o_vmem[pl.ds(a, n), c0:c0 + nc] = p.astype(o_vmem.dtype)
            elif kind == "w_sums":
                for q in range(0, h, _T_ROWS):
                    b11 = w_vmem[q:q + _T_ROWS, 0:h].astype(f32)
                    b12 = w_vmem[q:q + _T_ROWS, h:d].astype(f32)
                    b21 = w_vmem[h + q:h + q + _T_ROWS, 0:h].astype(f32)
                    b22 = w_vmem[h + q:h + q + _T_ROWS, h:d].astype(f32)
                    for k, t in enumerate((b11 + b22, b12 - b22, b21 - b11, b11 + b12, b21 + b22)):
                        t_vmem[k, q:q + _T_ROWS, :] = t.astype(mxu)
            elif kind == "norm_sums":
                _, a, n = step
                half = n // 2
                for q in range(0, half, _PREP_ROWS):
                    top = norm(a + q, _PREP_ROWS)
                    bot = norm(a + half + q, _PREP_ROWS)
                    a11, a12, a21, a22 = top[:, :h], top[:, h:], bot[:, :h], bot[:, h:]
                    for k, s in enumerate((a11 + a22, a21 + a22, a11, a22,
                                           a11 + a12, a21 - a11, a12 - a22)):
                        s_vmem[k, pl.ds(a // 2 + q, _PREP_ROWS), :] = s.astype(mxu)
            elif kind == "strassen":
                _, a, n = step
                half = n // 2

                def prod(k, rhs):
                    return jnp.dot(s_vmem[k, pl.ds(a // 2, half), :], rhs,
                                   preferred_element_type=f32)

                m1 = prod(0, t_vmem[0])
                m2 = prod(1, w_vmem[0:h, 0:h])
                m3 = prod(2, t_vmem[1])
                m4 = prod(3, t_vmem[2])
                m5 = prod(4, w_vmem[h:d, h:d])
                m6 = prod(5, t_vmem[3])
                m7 = prod(6, t_vmem[4])
                o_vmem[pl.ds(a, half), 0:h] = (m1 + m4 - m5 + m7).astype(o_vmem.dtype)
                o_vmem[pl.ds(a, half), h:d] = (m3 + m5).astype(o_vmem.dtype)
                o_vmem[pl.ds(a + half, half), 0:h] = (m2 + m4).astype(o_vmem.dtype)
                o_vmem[pl.ds(a + half, half), h:d] = (m1 - m2 + m3 + m6).astype(o_vmem.dtype)
            else:
                raise ValueError(kind)

    out = pl.pallas_call(
        kernel_function,
        in_specs=[pl.BlockSpec(memory_space=pl.ANY)] * 4,
        out_specs=pl.BlockSpec(memory_space=pl.ANY),
        out_shape=jax.ShapeDtypeStruct((m, d), x.dtype),
        scratch_shapes=[
            pltpu.VMEM((m, d), x.dtype),
            pltpu.VMEM((d, d), w.dtype),
            pltpu.VMEM((m, d), mxu),
            pltpu.VMEM((m, d), x.dtype),
            pltpu.VMEM((r0, d), f32),
            pltpu.VMEM((5, h, h), mxu),
            pltpu.VMEM((7, m // 2, h), mxu),
            pltpu.VMEM((d,), g.dtype),
            pltpu.VMEM((d,), b.dtype),
            pltpu.SemaphoreType.DMA((n_x,)),
            pltpu.SemaphoreType.DMA((len(_WK),)),
            pltpu.SemaphoreType.DMA((n_out,)),
            pltpu.SemaphoreType.DMA((2,)),
        ],
        compiler_params=pltpu.CompilerParams(
            vmem_limit_bytes=110 * 1024 * 1024,
            flags={"XLA_TPU_EVENLY_DISTRIBUTE_CRITICAL_NODES": True},
        ),
    )(x.reshape(m, d), g, b, w)
    return out.reshape(bsz, seq, d)
```
